```python
import os as _os
_os.environ.setdefault('JAX_PLATFORMS', 'cpu')
import jax
import jax.numpy as jnp

def _softmax(x, axis=-1):
    return jax.nn.softmax(x, axis=axis)

def _gelu(x):
    return jax.nn.gelu(x, approximate=True)

def _silu(x):
    return jax.nn.silu(x)

def _sigmoid(x):
    return jax.nn.sigmoid(x)

def _layernorm(x, axis=-1, eps=1e-05):
    m = jnp.mean(x, axis=axis, keepdims=True)
    v = jnp.var(x, axis=axis, keepdims=True)
    return (x - m) / jnp.sqrt(v + eps)

def _scatter_add(tgt, idx, src, axis=0):
    return tgt.at[idx].add(src)

def _segment_sum(src, seg, n):
    return jax.ops.segment_sum(src, seg, n)

class _Rng:

    def __init__(self, key):
        self._k = key

    def _next(self):
        self._k, sub = jax.random.split(self._k)
        return sub

    def normal(self, shape):
        return jax.random.normal(self._next(), shape, dtype=jnp.bfloat16)

    def randint(self, lo, hi, shape):
        return jax.random.randint(self._next(), shape, lo, hi, dtype=jnp.int32)

    def uniform(self, shape, lo=0.0, hi=1.0):
        return jax.random.uniform(self._next(), shape, jnp.bfloat16, lo, hi)

    def permutation(self, n):
        return jax.random.permutation(self._next(), n)
kernel_name = 'adaLN_cond__sliding_local_dilated__dense_activation_relu__prompt'

def setup_inputs():
    _rng = _Rng(jax.random.key(int.from_bytes(__import__("os").urandom(4), "little")))
    _w = lambda a: (lambda t: t.astype(jnp.bfloat16) if jnp.issubdtype(t.dtype, jnp.floating) else t)(jnp.asarray(a))

    def _A_setup():
        B, S, D = (1, 2048, 576)
        return {'x': _w((lambda *s: _rng.normal(s) * 0.05)(B, S, D)), 'wqkv': _w((lambda *s: _rng.normal(s) * 0.05)(D, 3 * D)), 'wo': _w((lambda *s: _rng.normal(s) * 0.05)(D, D))}
    _A_in = _A_setup()

    def _B_setup():
        B, S, D, Dff = (1, 2048, 576, 4608)
        return {'x': _w((lambda *s: _rng.normal(s) * 0.05)(B, S, D)), 'w1': _w((lambda *s: _rng.normal(s) * 0.05)(D, Dff)), 'w2': _w((lambda *s: _rng.normal(s) * 0.05)(Dff, D))}
    _B_in = _B_setup()
    return {'A_x': _A_in['x'], 'A_wqkv': _A_in['wqkv'], 'A_wo': _A_in['wo'], 'B_x': _B_in['x'], 'B_w1': _B_in['w1'], 'B_w2': _B_in['w2'], 'c': _w((lambda *s: _rng.normal(s) * 0.05)(1, 576) * 8.0), 'w_mod': _w((lambda *s: _rng.normal(s) * 0.05)(576, 6 * 576) * 576 ** (-0.5) * 8.0)}

def reference(A_x, A_wqkv, A_wo, B_x, B_w1, B_w2, c, w_mod):

    def _A_ref(x, wqkv, wo):
        B, S, D = x.shape
        H = 32
        Dh = D // H
        W, dil = (8, 2)
        qkv = (lambda x, *d: x.transpose(*d))((x @ wqkv).reshape(B, S, 3, H, Dh), 2, 0, 3, 1, 4)
        q, k, v = (qkv[0], qkv[1], qkv[2])
        scale = Dh ** (-0.5)
        pos = jnp.arange(S)
        off = jnp.arange(W) * dil
        idx = pos[:, None] - off[None, :]
        mask = idx >= 0
        idx_c = jnp.where(mask, idx, 0).reshape(-1)
        kg = k[:, :, idx_c, :].reshape(B, H, S, W, Dh)
        vg = v[:, :, idx_c, :].reshape(B, H, S, W, Dh)
        logits = jnp.einsum('bhsd,bhswd->bhsw', q, kg) * scale
        logits = jnp.where(mask[None, None, :, :], logits, -1000000000.0)
        attn = _softmax(logits, axis=-1)
        o = jnp.einsum('bhsw,bhswd->bhsd', attn, vg)
        return (lambda x, *d: x.transpose(*d))(o, 0, 2, 1, 3).reshape(B, S, D) @ wo

    def _B_ref(x, w1, w2):
        h = jnp.einsum('bsd,df->bsf', x, w1)
        zero = jnp.zeros_like(h)
        h = jnp.maximum(h, zero)
        return jnp.einsum('bsf,fd->bsd', h, w2)
    x = A_x
    mod = (_silu(c) @ w_mod).reshape(c.shape[0], 6, 1, -1)
    sa, ca, ga, sb, cb, gb = (mod[:, 0].copy(), mod[:, 1].copy(), mod[:, 2].copy(), mod[:, 3].copy(), mod[:, 4].copy(), mod[:, 5].copy())
    h = _layernorm(x, axis=-1) * (1 + ca) + sa
    x = x + ga * _A_ref(h, A_wqkv, A_wo)
    h = _layernorm(x, axis=-1) * (1 + cb) + sb
    x = x + gb * _B_ref(h, B_w1, B_w2)
    return x
```

```python
import functools

import jax
import jax.numpy as jnp
import jax.experimental.pallas as pl
import jax.experimental.pallas.tpu as pltpu

_H = 32
_W = 8
_DIL = 2
_HALO = 16
_EPS = 1e-05


def _layernorm_f32(x):
    m = jnp.mean(x, axis=-1, keepdims=True)
    xc = x - m
    v = jnp.mean(xc * xc, axis=-1, keepdims=True)
    return xc * jax.lax.rsqrt(v + _EPS)


def _kernel(x_ref, c_ref, wmod_hbm, wqkv_hbm, wo_hbm, w1_hbm, w2_hbm, o_ref,
            wmod_v, wqkv_v, wo_v, w1_v, w2_v, wqkvp_v, wop_v, mod_v,
            q_v, k_v, v_v, att_v, sems, *, TM, D, DP, DFF, FC, R):
    step = pl.program_id(0)
    Dh = D // _H
    nfc = DFF // FC
    bf16 = jnp.bfloat16
    f32 = jnp.float32

    def cp_wmod():
        return pltpu.make_async_copy(wmod_hbm, wmod_v, sems.at[0])

    def cp_wqkv():
        return pltpu.make_async_copy(wqkv_hbm, wqkv_v, sems.at[1])

    def cp_wo():
        return pltpu.make_async_copy(wo_hbm, wo_v, sems.at[2])

    def cp_w1():
        return pltpu.make_async_copy(w1_hbm, w1_v, sems.at[3])

    def cp_w2():
        return pltpu.make_async_copy(w2_hbm, w2_v, sems.at[4])

    @pl.when(step == 0)
    def _prologue():
        cp_wmod().start()
        cp_wqkv().start()
        cp_wo().start()
        cp_w1().start()
        cp_w2().start()

        k_v[0:_HALO, :] = jnp.zeros((_HALO, DP), f32)
        v_v[0:_HALO, :] = jnp.zeros((_HALO, DP), f32)

        r_i = jax.lax.broadcasted_iota(jnp.int32, (D, DP), 0)
        c_i = jax.lax.broadcasted_iota(jnp.int32, (D, DP), 1)
        src = (c_i & (_H - 1)) * Dh + (c_i >> 5)
        perm = jnp.where((r_i == src) & (c_i < D), 1.0, 0.0).astype(bf16)
        r_t = jax.lax.broadcasted_iota(jnp.int32, (DP, D), 0)
        c_t = jax.lax.broadcasted_iota(jnp.int32, (DP, D), 1)
        src_t = (r_t & (_H - 1)) * Dh + (r_t >> 5)
        perm_t = jnp.where((c_t == src_t) & (r_t < D), 1.0, 0.0).astype(bf16)

        cp_wmod().wait()
        cc = c_ref[...].astype(f32)
        sc = (cc * jax.nn.sigmoid(cc)).astype(bf16)
        sc8 = jnp.broadcast_to(sc, (8, D))
        for p in range(6):
            mp = jnp.dot(sc8, wmod_v[:, p * D:(p + 1) * D],
                         preferred_element_type=f32)
            mp = mp.astype(bf16)
            if p in (1, 4):
                mp = (1.0 + mp.astype(f32)).astype(bf16)
            mod_v[p * 8:(p + 1) * 8, :] = mp.astype(f32)

        cp_wqkv().wait()
        for p in range(3):
            wqkvp_v[:, p * DP:(p + 1) * DP] = jnp.dot(
                wqkv_v[:, p * D:(p + 1) * D], perm,
                preferred_element_type=f32).astype(bf16)
        cp_wo().wait()
        wop_v[...] = jnp.dot(perm_t, wo_v[...],
                             preferred_element_type=f32).astype(bf16)

    sa = mod_v[0:1, :]
    ca1 = mod_v[8:9, :]
    ga = mod_v[16:17, :]
    sb = mod_v[24:25, :]
    cb1 = mod_v[32:33, :]
    gb = mod_v[40:41, :]

    x = x_ref[...].astype(f32)
    h = (_layernorm_f32(x) * ca1 + sa).astype(bf16)
    qkv = jnp.dot(h, wqkvp_v[...], preferred_element_type=f32)
    q_v[...] = qkv[:, 0:DP]
    k_v[_HALO:_HALO + TM, :] = qkv[:, DP:2 * DP]
    v_v[_HALO:_HALO + TM, :] = qkv[:, 2 * DP:3 * DP]

    scale = float(Dh) ** -0.5
    nlt = DP // 128
    row0 = step * TM

    def attn_chunk(ci, carry):
        base = pl.multiple_of(ci * R, R)
        q = q_v[pl.ds(base, R), :]
        kwin = k_v[pl.ds(base, R + _HALO), :]
        pos = row0 + base + jax.lax.broadcasted_iota(jnp.int32, (R, 128), 0)
        logits = []
        for w in range(_W):
            off = _HALO - _DIL * w
            p = q * kwin[off:off + R, :]
            t = p[:, 0:128]
            for j in range(1, nlt):
                t = t + p[:, j * 128:(j + 1) * 128]
            t = t + pltpu.roll(t, 64, 1)
            t = t + pltpu.roll(t, 32, 1)
            t = t * scale
            if w > 0:
                t = jnp.where(pos >= _DIL * w, t, -1000000000.0)
            logits.append(t)
        m = logits[0]
        for w in range(1, _W):
            m = jnp.maximum(m, logits[w])
        es = [jnp.exp(l - m) for l in logits]
        den = es[0]
        for w in range(1, _W):
            den = den + es[w]
        inv = 1.0 / den
        vwin = v_v[pl.ds(base, R + _HALO), :]
        acc = [None] * nlt
        for w in range(_W):
            off = _HALO - _DIL * w
            a = es[w] * inv
            vs = vwin[off:off + R, :]
            for j in range(nlt):
                term = a * vs[:, j * 128:(j + 1) * 128]
                acc[j] = term if acc[j] is None else acc[j] + term
        att_v[pl.ds(base, R), :] = jnp.concatenate(acc, axis=1).astype(bf16)
        return carry

    jax.lax.fori_loop(0, TM // R, attn_chunk, 0)

    k_v[0:_HALO, :] = k_v[TM:TM + _HALO, :]
    v_v[0:_HALO, :] = v_v[TM:TM + _HALO, :]

    att = jnp.dot(att_v[...], wop_v[...], preferred_element_type=f32)
    x1 = x + ga * att

    @pl.when(step == 0)
    def _wait_ffn_weights():
        cp_w1().wait()
        cp_w2().wait()

    h2 = (_layernorm_f32(x1) * cb1 + sb).astype(bf16)
    acc = jnp.zeros((TM, D), f32)
    for ci in range(nfc):
        hc = jnp.dot(h2, w1_v[:, ci * FC:(ci + 1) * FC], preferred_element_type=f32)
        hc = jnp.maximum(hc, 0.0).astype(bf16)
        acc = acc + jnp.dot(hc, w2_v[ci * FC:(ci + 1) * FC, :],
                            preferred_element_type=f32)
    o_ref[...] = (x1 + gb * acc).astype(o_ref.dtype)


@jax.jit
def pallas_adaLN_cond__sliding_local_dilated__dense_activation_relu__prompt_kernel(
    A_x: jax.Array,
    A_wqkv: jax.Array,
    A_wo: jax.Array,
    B_x: jax.Array,
    B_w1: jax.Array,
    B_w2: jax.Array,
    c: jax.Array,
    w_mod: jax.Array,
):
    B, S, D = A_x.shape
    assert B == 1
    DFF = B_w1.shape[1]
    DP = ((D + 127) // 128) * 128
    TM = 512
    FC = 512
    R = 8
    bf16 = jnp.bfloat16
    f32 = jnp.float32

    x2 = A_x.reshape(S, D)

    kern = functools.partial(_kernel, TM=TM, D=D, DP=DP, DFF=DFF, FC=FC, R=R)
    any_spec = pl.BlockSpec(memory_space=pl.ANY)
    out = pl.pallas_call(
        kern,
        grid=(S // TM,),
        in_specs=[
            pl.BlockSpec((TM, D), lambda i: (i, 0)),
            pl.BlockSpec((1, D), lambda i: (0, 0)),
            any_spec, any_spec, any_spec, any_spec, any_spec,
        ],
        out_specs=pl.BlockSpec((TM, D), lambda i: (i, 0)),
        out_shape=jax.ShapeDtypeStruct((S, D), A_x.dtype),
        scratch_shapes=[
            pltpu.VMEM((D, 6 * D), bf16),
            pltpu.VMEM((D, 3 * D), bf16),
            pltpu.VMEM((D, D), bf16),
            pltpu.VMEM((D, DFF), bf16),
            pltpu.VMEM((DFF, D), bf16),
            pltpu.VMEM((D, 3 * DP), bf16),
            pltpu.VMEM((DP, D), bf16),
            pltpu.VMEM((48, D), f32),
            pltpu.VMEM((TM, DP), f32),
            pltpu.VMEM((TM + _HALO, DP), f32),
            pltpu.VMEM((TM + _HALO, DP), f32),
            pltpu.VMEM((TM, DP), bf16),
            pltpu.SemaphoreType.DMA((5,)),
        ],
        compiler_params=pltpu.CompilerParams(
            dimension_semantics=("arbitrary",),
            vmem_limit_bytes=100 * 1024 * 1024,
        ),
    )(x2, c, w_mod, A_wqkv, A_wo, B_w1, B_w2)
    return out.reshape(B, S, D)
```

```python
import functools

import jax
import jax.numpy as jnp
import jax.experimental.pallas as pl
import jax.experimental.pallas.tpu as pltpu

_H = 32
_W = 8
_DIL = 2
_HALO = 16
_EPS = 1e-05
_NEG = -1000000000.0


def _layernorm_f32(x):
    m = jnp.mean(x, axis=-1, keepdims=True)
    xc = x - m
    v = jnp.mean(xc * xc, axis=-1, keepdims=True)
    return xc * jax.lax.rsqrt(v + _EPS)


def _kernel(xt_ref, c_ref, wmod_hbm, wqkv_hbm, wo_hbm, w1_hbm, w2t_hbm, ot_ref,
            wmod_v, wqkv_v, wo_v, w1_v, w2t_v, wqkvp_v, wop_v, mod_v,
            q_v, k_v, v_v, att_v, x_v, h2_v, acc_v, x1t_v, gbt_v, sems, wsems,
            *, TM, D, DP, DFF, NCH, R, nblk):
    step = pl.program_id(0)
    Dh = D // _H
    FC = DFF // NCH
    RA = TM // NCH
    bf16 = jnp.bfloat16
    f32 = jnp.float32

    def cp_wmod_a():
        return pltpu.make_async_copy(wmod_hbm.at[:, 0:2 * D], wmod_v.at[:, 0:2 * D], sems.at[0])

    def cp_wmod_b():
        return pltpu.make_async_copy(wmod_hbm.at[:, 2 * D:6 * D], wmod_v.at[:, 2 * D:6 * D], sems.at[1])

    def cp_wqkv():
        return pltpu.make_async_copy(wqkv_hbm, wqkv_v, sems.at[2])

    def cp_wo():
        return pltpu.make_async_copy(wo_hbm, wo_v, sems.at[3])

    def cp_w1(ci):
        return pltpu.make_async_copy(w1_hbm.at[:, ci * FC:(ci + 1) * FC], w1_v.at[ci], wsems.at[0, ci])

    def cp_w2(ci):
        return pltpu.make_async_copy(w2t_hbm.at[:, ci * FC:(ci + 1) * FC], w2t_v.at[ci], wsems.at[1, ci])

    def silu_c8():
        cc = c_ref[...].astype(f32)
        sc = (cc * jax.nn.sigmoid(cc)).astype(bf16)
        return jnp.broadcast_to(sc, (8, D))

    def mod_part(p, sc8):
        mp = jnp.dot(sc8, wmod_v[:, p * D:(p + 1) * D], preferred_element_type=f32)
        mp = mp.astype(bf16)
        if p in (1, 4):
            mp = (1.0 + mp.astype(f32)).astype(bf16)
        mod_v[p * 8:(p + 1) * 8, :] = mp.astype(f32)

    @pl.when(step == 0)
    def _prologue():
        cp_wmod_a().start()
        cp_wqkv().start()

        k_v[0:_HALO, :] = jnp.zeros((_HALO, DP), f32)
        v_v[0:_HALO, :] = jnp.zeros((_HALO, DP), f32)

        r_i = jax.lax.broadcasted_iota(jnp.int32, (D, DP), 0)
        c_i = jax.lax.broadcasted_iota(jnp.int32, (D, DP), 1)
        src = (c_i & (_H - 1)) * Dh + (c_i >> 5)
        perm = jnp.where((r_i == src) & (c_i < D), 1.0, 0.0).astype(bf16)

        sc8 = silu_c8()
        cp_wmod_a().wait()
        cp_wo().start()
        cp_wmod_b().start()
        mod_part(0, sc8)
        mod_part(1, sc8)

        cp_wqkv().wait()
        for ci in range(NCH):
            cp_w1(ci).start()
            cp_w2(ci).start()
        for p in range(3):
            wqkvp_v[:, p * DP:(p + 1) * DP] = jnp.dot(
                wqkv_v[:, p * D:(p + 1) * D], perm,
                preferred_element_type=f32).astype(bf16)

    scale = float(Dh) ** -0.5
    nlt = DP // 128
    row0 = step * TM

    def ln1_qkv():
        x = xt_ref[...].astype(f32).T
        x_v[...] = x
        h = (_layernorm_f32(x) * mod_v[8:9, :] + mod_v[0:1, :]).astype(bf16)
        qkv = jnp.dot(h, wqkvp_v[...], preferred_element_type=f32)
        q_v[...] = qkv[:, 0:DP]
        k_v[_HALO:_HALO + TM, :] = qkv[:, DP:2 * DP]
        v_v[_HALO:_HALO + TM, :] = qkv[:, 2 * DP:3 * DP]

    def attn_rows(base):
        q = q_v[base:base + R, :]
        kwin = k_v[base:base + R + _HALO, :]
        pos = row0 + base + jax.lax.broadcasted_iota(jnp.int32, (R, 128), 0)
        logits = []
        for w in range(_W):
            off = _HALO - _DIL * w
            p = q * kwin[off:off + R, :]
            t = p[:, 0:128]
            for j in range(1, nlt):
                t = t + p[:, j * 128:(j + 1) * 128]
            t = t + pltpu.roll(t, 64, 1)
            t = t + pltpu.roll(t, 32, 1)
            t = t * scale
            if w > 0:
                t = jnp.where(pos >= _DIL * w, t, _NEG)
            logits.append(t)
        m = logits[0]
        for w in range(1, _W):
            m = jnp.maximum(m, logits[w])
        es = [jnp.exp(l - m) for l in logits]
        den = es[0]
        for w in range(1, _W):
            den = den + es[w]
        inv = 1.0 / den
        vwin = v_v[base:base + R + _HALO, :]
        acc = [None] * nlt
        for w in range(_W):
            off = _HALO - _DIL * w
            a = es[w] * inv
            vs = vwin[off:off + R, :]
            for j in range(nlt):
                term = a * vs[:, j * 128:(j + 1) * 128]
                acc[j] = term if acc[j] is None else acc[j] + term
        att_v[base:base + R, :] = jnp.concatenate(acc, axis=1).astype(bf16)

    def attn_part(ci):
        for r in range(RA // R):
            attn_rows(ci * RA + r * R)

    def ffn_part(ci):
        hc = jnp.dot(h2_v[...], w1_v[ci], preferred_element_type=f32)
        hc = jnp.maximum(hc, 0.0).astype(bf16)
        acc_v[...] += jax.lax.dot_general(
            w2t_v[ci], hc, (((1,), (1,)), ((), ())), preferred_element_type=f32)

    def write_out():
        gbt = jnp.concatenate([gbt_v[...]] * (TM // 128), axis=1)
        ot_ref[...] = (x1t_v[...] + gbt * acc_v[...]).astype(ot_ref.dtype)

    def wo_ln2():
        k_v[0:_HALO, :] = k_v[TM:TM + _HALO, :]
        v_v[0:_HALO, :] = v_v[TM:TM + _HALO, :]
        att = jnp.dot(att_v[...], wop_v[...], preferred_element_type=f32)
        x1 = x_v[...] + mod_v[16:17, :] * att
        x1t_v[...] = x1.T
        h2_v[...] = (_layernorm_f32(x1) * mod_v[32:33, :] + mod_v[24:25, :]).astype(bf16)
        acc_v[...] = jnp.zeros((D, TM), f32)

    @pl.when(step == 0)
    def _first_step():
        ln1_qkv()
        sc8 = silu_c8()
        r_t = jax.lax.broadcasted_iota(jnp.int32, (DP, D), 0)
        c_t = jax.lax.broadcasted_iota(jnp.int32, (DP, D), 1)
        src_t = (r_t & (_H - 1)) * Dh + (r_t >> 5)
        perm_t = jnp.where((c_t == src_t) & (r_t < D), 1.0, 0.0).astype(bf16)
        cp_wmod_b().wait()
        cp_wo().wait()
        for p in range(2, 6):
            mod_part(p, sc8)
        gbt_v[...] = jnp.broadcast_to(mod_v[40:41, :], (128, D)).T
        wop_v[...] = jnp.dot(perm_t, wo_v[...], preferred_element_type=f32).astype(bf16)
        for ci in range(NCH):
            attn_part(ci)
        wo_ln2()
        for ci in range(NCH):
            cp_w1(ci).wait()
            cp_w2(ci).wait()

    @pl.when(jnp.logical_and(step > 0, step < nblk))
    def _mid_step():
        ffn_part(0)
        ln1_qkv()
        for ci in range(1, NCH):
            ffn_part(ci)
            attn_part(ci - 1)
        attn_part(NCH - 1)
        write_out()
        wo_ln2()

    @pl.when(step == nblk)
    def _last_step():
        for ci in range(NCH):
            ffn_part(ci)
        write_out()


@jax.jit
def pallas_adaLN_cond__sliding_local_dilated__dense_activation_relu__prompt_kernel(
    A_x: jax.Array,
    A_wqkv: jax.Array,
    A_wo: jax.Array,
    B_x: jax.Array,
    B_w1: jax.Array,
    B_w2: jax.Array,
    c: jax.Array,
    w_mod: jax.Array,
):
    B, S, D = A_x.shape
    assert B == 1
    DFF = B_w1.shape[1]
    DP = ((D + 127) // 128) * 128
    TM = 256
    NCH = 2
    R = 32
    FC = DFF // NCH
    nblk = S // TM
    bf16 = jnp.bfloat16
    f32 = jnp.float32

    xt = A_x.reshape(S, D).T
    w2t = B_w2.T

    kern = functools.partial(_kernel, TM=TM, D=D, DP=DP, DFF=DFF, NCH=NCH, R=R, nblk=nblk)
    hbm_spec = pl.BlockSpec(memory_space=pltpu.HBM)
    out_t = pl.pallas_call(
        kern,
        grid=(nblk + 1,),
        in_specs=[
            pl.BlockSpec((D, TM), lambda i: (0, jnp.minimum(i, nblk - 1))),
            pl.BlockSpec((1, D), lambda i: (0, 0)),
            hbm_spec, hbm_spec, hbm_spec, hbm_spec, hbm_spec,
        ],
        out_specs=pl.BlockSpec((D, TM), lambda i: (0, jnp.maximum(i - 1, 0))),
        out_shape=jax.ShapeDtypeStruct((D, S), A_x.dtype),
        scratch_shapes=[
            pltpu.VMEM((D, 6 * D), bf16),
            pltpu.VMEM((D, 3 * D), bf16),
            pltpu.VMEM((D, D), bf16),
            pltpu.VMEM((NCH, D, FC), bf16),
            pltpu.VMEM((NCH, D, FC), bf16),
            pltpu.VMEM((D, 3 * DP), bf16),
            pltpu.VMEM((DP, D), bf16),
            pltpu.VMEM((48, D), f32),
            pltpu.VMEM((TM, DP), f32),
            pltpu.VMEM((TM + _HALO, DP), f32),
            pltpu.VMEM((TM + _HALO, DP), f32),
            pltpu.VMEM((TM, DP), bf16),
            pltpu.VMEM((TM, D), f32),
            pltpu.VMEM((TM, D), bf16),
            pltpu.VMEM((D, TM), f32),
            pltpu.VMEM((D, TM), f32),
            pltpu.VMEM((D, 128), f32),
            pltpu.SemaphoreType.DMA((4,)),
            pltpu.SemaphoreType.DMA((2, NCH)),
        ],
        compiler_params=pltpu.CompilerParams(
            dimension_semantics=("arbitrary",),
            vmem_limit_bytes=100 * 1024 * 1024,
        ),
    )(xt, c, w_mod, A_wqkv, A_wo, B_w1, w2t)
    return out_t.T.reshape(B, S, D)
```

```python
import functools

import jax
import jax.numpy as jnp
import jax.experimental.pallas as pl
import jax.experimental.pallas.tpu as pltpu

_H = 32
_W = 8
_DIL = 2
_HALO = 16
_EPS = 1e-05
_NEG = -1000000000.0


def _layernorm_f32(x):
    m = jnp.mean(x, axis=-1, keepdims=True)
    xc = x - m
    v = jnp.mean(xc * xc, axis=-1, keepdims=True)
    return xc * jax.lax.rsqrt(v + _EPS)


def _kernel(xt_ref, c_ref, wmod_hbm, wqkv_hbm, wo_hbm, w1_hbm, w2t_hbm, ot_ref,
            wmod_v, wqkv_v, wo_v, w1_v, w2t_v, wqkvp_v, wop_v, mod_v,
            q_v, k_v, v_v, att_v, x_v, h2_v, acc_v, x1t_v, gbt_v, sems, wsems,
            *, TM, D, DP, DFF, NCH, R, nblk):
    step = pl.program_id(0)
    Dh = D // _H
    FC = DFF // NCH
    RA = TM // NCH
    bf16 = jnp.bfloat16
    f32 = jnp.float32

    def cp_wmod_a():
        return pltpu.make_async_copy(wmod_hbm.at[:, 0:2 * D], wmod_v.at[:, 0:2 * D], sems.at[0])

    def cp_wmod_b():
        return pltpu.make_async_copy(wmod_hbm.at[:, 2 * D:6 * D], wmod_v.at[:, 2 * D:6 * D], sems.at[1])

    def cp_wqkv():
        return pltpu.make_async_copy(wqkv_hbm, wqkv_v, sems.at[2])

    def cp_wo():
        return pltpu.make_async_copy(wo_hbm, wo_v, sems.at[3])

    def cp_w1(ci):
        return pltpu.make_async_copy(w1_hbm.at[:, ci * FC:(ci + 1) * FC], w1_v.at[ci], wsems.at[0, ci])

    def cp_w2(ci):
        return pltpu.make_async_copy(w2t_hbm.at[:, ci * FC:(ci + 1) * FC], w2t_v.at[ci], wsems.at[1, ci])

    def silu_c8():
        cc = c_ref[...].astype(f32)
        sc = (cc * jax.nn.sigmoid(cc)).astype(bf16)
        return jnp.broadcast_to(sc, (8, D))

    def mod_part(p, sc8):
        mp = jnp.dot(sc8, wmod_v[:, p * D:(p + 1) * D], preferred_element_type=f32)
        mp = mp.astype(bf16)
        if p in (1, 4):
            mp = (1.0 + mp.astype(f32)).astype(bf16)
        mod_v[p * 8:(p + 1) * 8, :] = mp.astype(f32)

    @pl.when(step == 0)
    def _prologue():
        cp_wmod_a().start()
        cp_wqkv().start()

        k_v[0:_HALO, :] = jnp.zeros((_HALO, DP), f32)
        v_v[0:_HALO, :] = jnp.zeros((_HALO, DP), f32)

        r_i = jax.lax.broadcasted_iota(jnp.int32, (D, DP), 0)
        c_i = jax.lax.broadcasted_iota(jnp.int32, (D, DP), 1)
        src = (c_i & (_H - 1)) * Dh + (c_i >> 5)
        perm = jnp.where((r_i == src) & (c_i < D), 1.0, 0.0).astype(bf16)

        sc8 = silu_c8()
        cp_wmod_a().wait()
        cp_wo().start()
        cp_wmod_b().start()
        mod_part(0, sc8)
        mod_part(1, sc8)

        cp_wqkv().wait()
        for ci in range(NCH):
            cp_w1(ci).start()
            cp_w2(ci).start()
        for p in range(3):
            wqkvp_v[:, p * DP:(p + 1) * DP] = jnp.dot(
                wqkv_v[:, p * D:(p + 1) * D], perm,
                preferred_element_type=f32).astype(bf16)

    scale = float(Dh) ** -0.5
    nlt = DP // 128
    row0 = step * TM

    def ln1_qkv():
        x = xt_ref[...].astype(f32).T
        x_v[...] = x
        h = (_layernorm_f32(x) * mod_v[8:9, :] + mod_v[0:1, :]).astype(bf16)
        qkv = jnp.dot(h, wqkvp_v[...], preferred_element_type=f32)
        q_v[...] = qkv[:, 0:DP]
        k_v[_HALO:_HALO + TM, :] = qkv[:, DP:2 * DP]
        v_v[_HALO:_HALO + TM, :] = qkv[:, 2 * DP:3 * DP]

    def attn_rows(base):
        q = q_v[pl.ds(base, R), :]
        kwin = k_v[pl.ds(base, R + _HALO), :]
        pos = row0 + base + jax.lax.broadcasted_iota(jnp.int32, (R, 128), 0)
        logits = []
        for w in range(_W):
            off = _HALO - _DIL * w
            p = q * kwin[off:off + R, :]
            t = p[:, 0:128]
            for j in range(1, nlt):
                t = t + p[:, j * 128:(j + 1) * 128]
            t = t + pltpu.roll(t, 64, 1)
            t = t + pltpu.roll(t, 32, 1)
            t = t * scale
            if w > 0:
                t = jnp.where(pos >= _DIL * w, t, _NEG)
            logits.append(t)
        m = logits[0]
        for w in range(1, _W):
            m = jnp.maximum(m, logits[w])
        es = [jnp.exp(l - m) for l in logits]
        den = es[0]
        for w in range(1, _W):
            den = den + es[w]
        inv = 1.0 / den
        vwin = v_v[pl.ds(base, R + _HALO), :]
        acc = [None] * nlt
        for w in range(_W):
            off = _HALO - _DIL * w
            a = es[w] * inv
            vs = vwin[off:off + R, :]
            for j in range(nlt):
                term = a * vs[:, j * 128:(j + 1) * 128]
                acc[j] = term if acc[j] is None else acc[j] + term
        att_v[pl.ds(base, R), :] = jnp.concatenate(acc, axis=1).astype(bf16)

    def attn_part(ci):
        for r in range(RA // R):
            attn_rows(ci * RA + r * R)

    def ffn_part(ci):
        hc = jnp.dot(h2_v[...], w1_v[ci], preferred_element_type=f32)
        hc = jnp.maximum(hc, 0.0).astype(bf16)
        acc_v[...] += jax.lax.dot_general(
            w2t_v[ci], hc, (((1,), (1,)), ((), ())), preferred_element_type=f32)

    def write_out():
        gbt = jnp.concatenate([gbt_v[...]] * (TM // 128), axis=1)
        ot_ref[...] = (x1t_v[...] + gbt * acc_v[...]).astype(ot_ref.dtype)

    def wo_ln2():
        k_v[0:_HALO, :] = k_v[TM:TM + _HALO, :]
        v_v[0:_HALO, :] = v_v[TM:TM + _HALO, :]
        att = jnp.dot(att_v[...], wop_v[...], preferred_element_type=f32)
        x1 = x_v[...] + mod_v[16:17, :] * att
        x1t_v[...] = x1.T
        h2_v[...] = (_layernorm_f32(x1) * mod_v[32:33, :] + mod_v[24:25, :]).astype(bf16)
        acc_v[...] = jnp.zeros((D, TM), f32)

    @pl.when(step == 0)
    def _first_step():
        ln1_qkv()
        sc8 = silu_c8()
        r_t = jax.lax.broadcasted_iota(jnp.int32, (DP, D), 0)
        c_t = jax.lax.broadcasted_iota(jnp.int32, (DP, D), 1)
        src_t = (r_t & (_H - 1)) * Dh + (r_t >> 5)
        perm_t = jnp.where((c_t == src_t) & (r_t < D), 1.0, 0.0).astype(bf16)
        cp_wmod_b().wait()
        cp_wo().wait()
        for p in range(2, 6):
            mod_part(p, sc8)
        gbt_v[...] = jnp.broadcast_to(mod_v[40:41, :], (128, D)).T
        wop_v[...] = jnp.dot(perm_t, wo_v[...], preferred_element_type=f32).astype(bf16)

        def attn_body(r, carry):
            attn_rows(pl.multiple_of(r * R, R))
            return carry
        jax.lax.fori_loop(0, TM // R, attn_body, 0)
        wo_ln2()
        for ci in range(NCH):
            cp_w1(ci).wait()
            cp_w2(ci).wait()

    @pl.when(jnp.logical_and(step > 0, step < nblk))
    def _mid_step():
        ffn_part(0)
        ln1_qkv()
        for ci in range(1, NCH):
            ffn_part(ci)
            attn_part(ci - 1)
        attn_part(NCH - 1)
        write_out()
        wo_ln2()

    @pl.when(step == nblk)
    def _last_step():
        def ffn_body(ci, carry):
            ffn_part(ci)
            return carry
        jax.lax.fori_loop(0, NCH, ffn_body, 0)
        write_out()


@jax.jit
def pallas_adaLN_cond__sliding_local_dilated__dense_activation_relu__prompt_kernel(
    A_x: jax.Array,
    A_wqkv: jax.Array,
    A_wo: jax.Array,
    B_x: jax.Array,
    B_w1: jax.Array,
    B_w2: jax.Array,
    c: jax.Array,
    w_mod: jax.Array,
):
    B, S, D = A_x.shape
    assert B == 1
    DFF = B_w1.shape[1]
    DP = ((D + 127) // 128) * 128
    TM = 256
    NCH = 2
    R = 32
    FC = DFF // NCH
    nblk = S // TM
    bf16 = jnp.bfloat16
    f32 = jnp.float32

    xt = A_x.reshape(S, D).T
    w2t = B_w2.T

    kern = functools.partial(_kernel, TM=TM, D=D, DP=DP, DFF=DFF, NCH=NCH, R=R, nblk=nblk)
    hbm_spec = pl.BlockSpec(memory_space=pltpu.HBM)
    out_t = pl.pallas_call(
        kern,
        grid=(nblk + 1,),
        in_specs=[
            pl.BlockSpec((D, TM), lambda i: (0, jnp.minimum(i, nblk - 1))),
            pl.BlockSpec((1, D), lambda i: (0, 0)),
            hbm_spec, hbm_spec, hbm_spec, hbm_spec, hbm_spec,
        ],
        out_specs=pl.BlockSpec((D, TM), lambda i: (0, jnp.maximum(i - 1, 0))),
        out_shape=jax.ShapeDtypeStruct((D, S), A_x.dtype),
        scratch_shapes=[
            pltpu.VMEM((D, 6 * D), bf16),
            pltpu.VMEM((D, 3 * D), bf16),
            pltpu.VMEM((D, D), bf16),
            pltpu.VMEM((NCH, D, FC), bf16),
            pltpu.VMEM((NCH, D, FC), bf16),
            pltpu.VMEM((D, 3 * DP), bf16),
            pltpu.VMEM((DP, D), bf16),
            pltpu.VMEM((48, D), f32),
            pltpu.VMEM((TM, DP), f32),
            pltpu.VMEM((TM + _HALO, DP), f32),
            pltpu.VMEM((TM + _HALO, DP), f32),
            pltpu.VMEM((TM, DP), bf16),
            pltpu.VMEM((TM, D), f32),
            pltpu.VMEM((TM, D), bf16),
            pltpu.VMEM((D, TM), f32),
            pltpu.VMEM((D, TM), f32),
            pltpu.VMEM((D, 128), f32),
            pltpu.SemaphoreType.DMA((4,)),
            pltpu.SemaphoreType.DMA((2, NCH)),
        ],
        compiler_params=pltpu.CompilerParams(
            dimension_semantics=("arbitrary",),
            vmem_limit_bytes=100 * 1024 * 1024,
        ),
    )(xt, c, w_mod, A_wqkv, A_wo, B_w1, w2t)
    return out_t.T.reshape(B, S, D)
```
